```python
import jax
import jax.numpy as jnp

def _softmax(x, axis=-1):
    return jax.nn.softmax(x, axis=axis)
def _gelu(x):
    return jax.nn.gelu(x, approximate=True)
def _silu(x):
    return jax.nn.silu(x)
def _sigmoid(x):
    return jax.nn.sigmoid(x)
def _layernorm(x, axis=-1, eps=1e-5):
    m = jnp.mean(x, axis=axis, keepdims=True)
    v = jnp.var(x, axis=axis, keepdims=True)
    return (x - m) / jnp.sqrt(v + eps)
def _scatter_add(tgt, idx, src, axis=0):
    return tgt.at[idx].add(src)
def _segment_sum(src, seg, n):
    return jax.ops.segment_sum(src, seg, n)
class _Rng:
    def __init__(self, key):
        self._k = key
    def _next(self):
        self._k, sub = jax.random.split(self._k)
        return sub
    def normal(self, shape):
        return jax.random.normal(self._next(), shape, dtype=jnp.bfloat16)
    def randint(self, lo, hi, shape):
        return jax.random.randint(self._next(), shape, lo, hi, dtype=jnp.int32)
    def uniform(self, shape, lo=0.0, hi=1.0):
        return jax.random.uniform(self._next(), shape, jnp.bfloat16, lo, hi)
    def permutation(self, n):
        return jax.random.permutation(self._next(), n)


kernel_name = 'standalone__sliding_block_cached__decode'

def _fwd_setup_inputs():
    _rng = _Rng(jax.random.key(int.from_bytes(__import__("os").urandom(4), "little")))
    _w = (lambda a: (lambda t: t.astype(jnp.bfloat16) if jnp.issubdtype(t.dtype, jnp.floating) else t)(jnp.asarray(a)))
    B, Sq, D = 2, 1, 640
    Hq, Hkv, Sk, Dh = 32, 32, 4096, 128
    assert Hq % Hkv == 0, (Hq, Hkv)
    return {
        "x": _w((lambda *s: _rng.normal(s) * 0.05)(B, Sq, D)),
        "k_cache": _w((lambda *s: _rng.normal(s) * 0.05)(B, Hkv, Sk, Dh)),
        "v_cache": _w((lambda *s: _rng.normal(s) * 0.05)(B, Hkv, Sk, Dh)),
        "wq": _w((lambda *s: _rng.normal(s) * 0.05)(D, Hq * Dh) * (D ** -0.5)),
        "wo": _w((lambda *s: _rng.normal(s) * 0.05)(Hq * Dh, D) * ((Hq * Dh) ** -0.5)),
    }

def _fwd_reference(x, k_cache, v_cache, wq, wo):
    B, Sq, D = x.shape
    Hq, Dh = 32, 128
    Hkv, Sk = k_cache.shape[1], k_cache.shape[2]
    W = min(4096, max(256, Sk // 4))
    rep = Hq // Hkv
    q = (lambda x, *d: x.transpose(*d))((x @ wq).reshape(B, Sq, Hq, Dh), 0, 2, 1, 3)
    k = jnp.repeat(k_cache[:, :, Sk - W:, :], rep, axis=1)
    v = jnp.repeat(v_cache[:, :, Sk - W:, :], rep, axis=1)
    scores = jnp.einsum("bhqd,bhkd->bhqk", q, k) * (Dh ** -0.5)
    p = _softmax(scores, axis=-1)
    o = jnp.einsum("bhqk,bhkd->bhqd", p, v)
    return (lambda x, *d: x.transpose(*d))(o, 0, 2, 1, 3).reshape(B, Sq, Hq * Dh) @ wo


def setup_inputs():
    _inp = _fwd_setup_inputs()
    _gk = jax.random.fold_in(jax.random.key(int.from_bytes(__import__("os").urandom(4), "little")), 2**31 - 1)
    _shapes = [[2, 1, 640]]
    _dtypes = ['bfloat16']
    _gks = jax.random.split(_gk, len(_shapes))
    _gs = [jax.random.normal(k, s, dtype=jnp.dtype(d)) * 0.05 for k, s, d in zip(_gks, _shapes, _dtypes)]
    _inp["grad_out"] = _gs[0]
    return _inp

def reference(x, k_cache, v_cache, wq, wo, grad_out):
    _const = dict()
    def _f(*_d):
        return _fwd_reference(**{'x': _d[0], 'k_cache': _d[1], 'v_cache': _d[2], 'wq': _d[3], 'wo': _d[4], **_const})
    _out, _vjp = jax.vjp(_f, x, k_cache, v_cache, wq, wo)
    _grads = _vjp(grad_out)
    _out0 = jnp.asarray(_out)
    return (_out0, *[jnp.asarray(_g) for _g in _grads])
```

```python
import functools

import jax
import jax.numpy as jnp
import numpy as np
from jax import lax
from jax.experimental import pallas as pl
from jax.experimental.pallas import tpu as pltpu

F32 = jnp.float32
BF16 = jnp.bfloat16
_NN = (((1,), (0,)), ((), ()))
_NT = (((1,), (1,)), ((), ()))

B, D, H, SK, DH = 2, 640, 32, 4096, 128
W = min(4096, max(256, SK // 4))
Z = SK - W
BH, HD = B * H, H * DH
SCALE = float(np.asarray(DH ** -0.5, dtype=BF16))

R_GROUPS = ((10, 4), (6, 4))
R_ROWS = 16
R_WIN = 32
R_TAIL = 11
WQ_V = 5
WQ_RC = 512
WO_RV, WO_RR = 4, 8

W_GROUPS = ((6, 6), (7, 4))
W_ROWS = 64
CALL = 12
PRE_CALLS = 3
STEP_CALLS = 2
WQ_WC = 1024
WO_WV, WO_WR = 8, 16

WQ_ROWS = D // WQ_V
N_GROUPS = sum(c for _, c in W_GROUPS)
CALLS_PER_GROUP = Z // (W_ROWS * CALL)
N_CALLS = 2 * N_GROUPS * CALLS_PER_GROUP

assert sum(s * c for s, c in R_GROUPS) == BH and sum(s * c for s, c in W_GROUPS) == BH
assert (WQ_ROWS // 8) * (HD // WQ_RC) == HD // (WO_RV * WO_RR) >= R_WIN >= R_TAIL
assert CALLS_PER_GROUP * CALL * W_ROWS == Z and W % W_ROWS == 0 and W % R_ROWS == 0
assert PRE_CALLS <= CALLS_PER_GROUP and PRE_CALLS + STEP_CALLS * H <= N_CALLS


def _dot(a, b, dims):
    return lax.dot_general(a, b, dims, preferred_element_type=F32)


def _round(x):
    return x.astype(BF16).astype(F32)


def _tile(i, size):
    return pl.ds(pl.multiple_of(i * size, size), size)


def _divmod(t, n):
    assert n & (n - 1) == 0
    return t >> (n.bit_length() - 1), t & (n - 1)


def _loop(lo, hi, fn):
    def body(t, carry):
        fn(t)
        return carry
    lax.fori_loop(lo, hi, body, 0)


def _kernel(x_hbm, k_hbm, v_hbm, wq_hbm, wo_hbm, g_hbm,
            out_hbm, dx_hbm, dk_hbm, dv_hbm, dwq_hbm, dwo_hbm,
            xbuf, gbuf, kbuf, vbuf, wqbuf, wobuf,
            outbuf, dxbuf, dkbuf, dvbuf, dwqbuf, dwobuf, zbuf, sems):
    rsem, wsem = sems.at[0], sems.at[1]

    def paced(c, priority=0):
        c.start(priority=priority)
        c.wait()

    def wq_read(t):
        r, c = _divmod(t, HD // WQ_RC)
        idx = (slice(None), _tile(r, 8), _tile(c, WQ_RC))
        return pltpu.make_async_copy(wq_hbm.at[idx], wqbuf.at[idx], rsem)

    def wo_read(t):
        idx = (slice(None), _tile(t, WO_RR))
        return pltpu.make_async_copy(wo_hbm.at[idx], wobuf.at[idx], rsem)

    def kv_read(src, dst, h0, size, t):
        g, r = _divmod(t, W // R_ROWS)
        heads = pl.ds(h0 + g * size, size)
        return pltpu.make_async_copy(
            src.at[heads, _tile(Z // R_ROWS + r, R_ROWS)], dst.at[heads, _tile(r, R_ROWS)], rsem)

    x_read = pltpu.make_async_copy(x_hbm, xbuf, rsem)
    g_read = pltpu.make_async_copy(g_hbm, gbuf, rsem)
    x_read.start(priority=0)
    g_read.start(priority=1)
    _loop(0, R_WIN, lambda t: (wq_read(t).start(priority=0), wo_read(t).start(priority=1)))
    zbuf[...] = jnp.zeros_like(zbuf)
    x_read.wait()
    g_read.wait()
    _loop(R_WIN, HD // (WO_RV * WO_RR), lambda t: (paced(wq_read(t), 0), paced(wo_read(t), 1)))
    h0 = 0
    for size, count in R_GROUPS:
        _loop(0, count * (W // R_ROWS),
              lambda t, h0=h0, size=size: (paced(kv_read(k_hbm, kbuf, h0, size, t), 0),
                                           paced(kv_read(v_hbm, vbuf, h0, size, t), 1)))
        h0 += size * count
    _loop(0, R_WIN, lambda t: wq_read(t).wait())
    _loop(0, R_WIN - R_TAIL, lambda t: wo_read(t).wait())

    def zero_write(arr, head0, size, chunk):
        return pltpu.make_async_copy(
            zbuf.at[pl.ds(0, size)], arr.at[pl.ds(head0, size), _tile(chunk, W_ROWS)], wsem)

    def window_head(t):
        return zero_write(dk_hbm, 0, W_GROUPS[0][0], t)

    def zero_call(c):
        group, part = _divmod(c, CALLS_PER_GROUP)
        g0 = 0
        for arr in (dk_hbm, dv_hbm):
            head0 = 0
            for size, count in W_GROUPS:
                @pl.when(jnp.logical_and(group >= g0, group < g0 + count))
                def _(arr=arr, g0=g0, head0=head0, size=size):
                    head = head0 + (group - g0) * size
                    _loop(0, CALL, lambda t: paced(zero_write(arr, head, size, part * CALL + t)))
                g0 += count
                head0 += size * count

    _loop(0, PRE_CALLS * CALL, lambda t: window_head(t).start())
    _loop(R_WIN - R_TAIL, R_WIN, lambda t: wo_read(t).wait())

    row_d = lax.broadcasted_iota(jnp.int32, (8, D), 0)
    row_w = lax.broadcasted_iota(jnp.int32, (8, W), 0)
    row_h = lax.broadcasted_iota(jnp.int32, (8, DH), 0)

    def spread(buf, nrows):
        t = buf[...].astype(F32)
        both = jnp.where(row_d % 2 == 0, jnp.broadcast_to(t[0:1], (8, D)), jnp.broadcast_to(t[1:2], (8, D)))
        return jnp.where(row_d < nrows, both, 0.0)

    x4, g4 = spread(xbuf, 4).astype(BF16), spread(gbuf, 4).astype(BF16)
    g2 = spread(gbuf, 2).astype(BF16)
    x2_t = spread(xbuf, 2).T.astype(BF16)

    def per_batch(rows, a, m0, m1, dims):
        return jnp.where(rows % 2 == 0, _dot(a, m0, dims), _dot(a, m1, dims))

    def pick(a, r):
        return jnp.where(row_h == r, a, 0.0).astype(BF16)

    def step(h, carry):
        out_acc, dx_acc = carry
        c0 = PRE_CALLS + h * STEP_CALLS
        for u in range(STEP_CALLS // 2):
            zero_call(c0 + u)

        col = _tile(h, DH)
        wq_h = wqbuf[:, :, col].reshape(D, DH)
        blk, sub = _divmod(h, HD // (WO_RV * DH))
        wo_h = wobuf[blk, _tile(sub, DH), :]
        k0, k1, v0, v1 = kbuf[h], kbuf[H + h], vbuf[h], vbuf[H + h]

        q = _round(_dot(x4, wq_h, _NN))
        do = _round(_dot(g4, wo_h, _NT))
        s = _round(_round(per_batch(row_w, q.astype(BF16), k0, k1, _NT)) * SCALE)
        dp = _round(per_batch(row_w, do.astype(BF16), v0, v1, _NT))
        e = _round(jnp.exp(_round(s - jnp.max(s, axis=1, keepdims=True))))
        z = _round(jnp.sum(e, axis=1, keepdims=True))
        p = _round(e / z)
        dz = _round(jnp.sum(_round(_round(dp * _round(1.0 / (z * z))) * e), axis=1, keepdims=True))
        ds = _round(_round(_round(_round(dp / z) - dz) * e) * SCALE)
        o = per_batch(row_h, p.astype(BF16), v0, v1, _NN).astype(BF16)
        dq = per_batch(row_h, ds.astype(BF16), k0, k1, _NN).astype(BF16)
        out_acc = out_acc + _dot(o, wo_h, _NN)
        dx_acc = dx_acc + _dot(dq, wq_h, _NT)

        for u in range(STEP_CALLS // 2, STEP_CALLS):
            zero_call(c0 + u)

        pd_t = jnp.where(row_w < 2, p, jnp.where(row_w < 4, ds, 0.0)).T.astype(BF16)
        dvbuf[h] = _dot(pd_t, pick(do, 0), _NN).astype(BF16)
        dvbuf[H + h] = _dot(pd_t, pick(do, 1), _NN).astype(BF16)
        dkbuf[h] = _dot(pd_t, pick(q, 2), _NN).astype(BF16)
        dkbuf[H + h] = _dot(pd_t, pick(q, 3), _NN).astype(BF16)
        dwqbuf[:, :, col] = _dot(x2_t, dq, _NN).astype(BF16).reshape(WQ_V, WQ_ROWS, DH)
        o_t = o.astype(F32).T.astype(BF16)
        blk, sub = _divmod(h, HD // (WO_WV * DH))
        dwobuf[blk, _tile(sub, DH), :] = _dot(o_t, g2, _NN).astype(BF16)
        return out_acc, dx_acc

    acc0 = jnp.zeros((8, D), F32)
    out_acc, dx_acc = lax.fori_loop(0, H, step, (acc0, acc0))
    outbuf[...] = out_acc[0:B].astype(BF16)
    dxbuf[...] = dx_acc[0:B].astype(BF16)

    def write(src, dst):
        paced(pltpu.make_async_copy(src, dst, wsem))

    def dwq_write(t):
        r, c = _divmod(t, HD // WQ_WC)
        idx = (slice(None), _tile(r, 8), _tile(c, WQ_WC))
        write(dwqbuf.at[idx], dwq_hbm.at[idx])

    def dwo_write(t):
        idx = (slice(None), _tile(t, WO_WR))
        write(dwobuf.at[idx], dwo_hbm.at[idx])

    def dkv_write(src, dst, h0, size, t):
        g, r = _divmod(t, W // W_ROWS)
        heads = pl.ds(h0 + g * size, size)
        write(src.at[heads, _tile(r, W_ROWS)], dst.at[heads, _tile(Z // W_ROWS + r, W_ROWS)])

    write(outbuf, out_hbm)
    write(dxbuf, dx_hbm)
    _loop(PRE_CALLS + STEP_CALLS * H, N_CALLS, zero_call)
    _loop(0, (WQ_ROWS // 8) * (HD // WQ_WC), dwq_write)
    _loop(0, HD // (WO_WV * WO_WR), dwo_write)
    for src, dst in ((dkbuf, dk_hbm), (dvbuf, dv_hbm)):
        h0 = 0
        for size, count in W_GROUPS:
            _loop(0, count * (W // W_ROWS), functools.partial(dkv_write, src, dst, h0, size))
            h0 += size * count
    _loop(0, PRE_CALLS * CALL, lambda t: window_head(t).wait())


@jax.jit
def pallas_standalone__sliding_block_cached__decode_kernel(
    x: jax.Array,
    k_cache: jax.Array,
    v_cache: jax.Array,
    wq: jax.Array,
    wo: jax.Array,
    grad_out: jax.Array,
):
    assert x.shape == (B, 1, D) and k_cache.shape == (B, H, SK, DH) and wq.shape == (D, HD)
    xs, kvs, win = (B, D), (BH, SK, DH), (BH, W, DH)
    wqs = (WQ_V, WQ_ROWS, HD)
    wo_rs, wo_ws = (WO_RV, HD // WO_RV, D), (WO_WV, HD // WO_WV, D)
    zeros = (max(size for size, _ in W_GROUPS), W_ROWS, DH)
    hbm = pl.BlockSpec(memory_space=pl.ANY)
    out, dx, dk, dv, dwq, dwo = pl.pallas_call(
        _kernel,
        out_shape=tuple(jax.ShapeDtypeStruct(s, BF16) for s in (xs, xs, kvs, kvs, wqs, wo_ws)),
        in_specs=[hbm] * 6,
        out_specs=(hbm,) * 6,
        scratch_shapes=[
            *(pltpu.VMEM(s, BF16) for s in (xs, xs, win, win, wqs, wo_rs)),
            *(pltpu.VMEM(s, BF16) for s in (xs, xs, win, win, wqs, wo_ws)),
            pltpu.VMEM(zeros, BF16),
            pltpu.SemaphoreType.DMA((2,)),
        ],
        compiler_params=pltpu.CompilerParams(vmem_limit_bytes=100 * 1024 * 1024),
    )(x.reshape(xs), k_cache.reshape(kvs), v_cache.reshape(kvs),
      wq.reshape(wqs), wo.reshape(wo_rs), grad_out.reshape(xs))
    return (out.reshape(x.shape), dx.reshape(x.shape), dk.reshape(k_cache.shape),
            dv.reshape(v_cache.shape), dwq.reshape(wq.shape), dwo.reshape(wo.shape))
```
